```python
import jax
import jax.numpy as jnp

def _softmax(x, axis=-1):
    return jax.nn.softmax(x, axis=axis)
def _gelu(x):
    return jax.nn.gelu(x, approximate=True)
def _silu(x):
    return jax.nn.silu(x)
def _sigmoid(x):
    return jax.nn.sigmoid(x)
def _layernorm(x, axis=-1, eps=1e-5):
    m = jnp.mean(x, axis=axis, keepdims=True)
    v = jnp.var(x, axis=axis, keepdims=True)
    return (x - m) / jnp.sqrt(v + eps)
def _scatter_add(tgt, idx, src, axis=0):
    return tgt.at[idx].add(src)
def _segment_sum(src, seg, n):
    return jax.ops.segment_sum(src, seg, n)
class _Rng:
    def __init__(self, key):
        self._k = key
    def _next(self):
        self._k, sub = jax.random.split(self._k)
        return sub
    def normal(self, shape):
        return jax.random.normal(self._next(), shape, dtype=jnp.bfloat16)
    def randint(self, lo, hi, shape):
        return jax.random.randint(self._next(), shape, lo, hi, dtype=jnp.int32)
    def uniform(self, shape, lo=0.0, hi=1.0):
        return jax.random.uniform(self._next(), shape, jnp.bfloat16, lo, hi)
    def permutation(self, n):
        return jax.random.permutation(self._next(), n)


kernel_name = 'sequential_preLN__sliding_block_cached__mixer_s_mlp__decode'

def setup_inputs():
    _rng = _Rng(jax.random.key(int.from_bytes(__import__("os").urandom(4), "little")))
    _w = (lambda a: (lambda t: t.astype(jnp.bfloat16) if jnp.issubdtype(t.dtype, jnp.floating) else t)(jnp.asarray(a)))
    def _A_setup():
        B, Sq, D = 1, 1, 640
        Hq, Hkv, Sk, Dh = 32, 32, 32768, 192
        assert Hq % Hkv == 0, (Hq, Hkv)
        return {
            "x": _w((lambda *s: _rng.normal(s) * 0.05)(B, Sq, D)),
            "k_cache": _w((lambda *s: _rng.normal(s) * 0.05)(B, Hkv, Sk, Dh)),
            "v_cache": _w((lambda *s: _rng.normal(s) * 0.05)(B, Hkv, Sk, Dh)),
            "wq": _w((lambda *s: _rng.normal(s) * 0.05)(D, Hq * Dh) * (D ** -0.5)),
            "wo": _w((lambda *s: _rng.normal(s) * 0.05)(Hq * Dh, D) * ((Hq * Dh) ** -0.5)),
        }
    _A_in = _A_setup()

    def _B_setup():
        B, S, D, F = 1, 1, 640, 1536
        return {
            "x":  _w((lambda *s: _rng.normal(s) * 0.05)(B, S, D)),
            "w1": _w((lambda *s: _rng.normal(s) * 0.05)(D, D) * (D ** -0.5)),
            "w2": _w((lambda *s: _rng.normal(s) * 0.05)(D, D) * (D ** -0.5)),
            "w3": _w((lambda *s: _rng.normal(s) * 0.05)(D, F) * (D ** -0.5)),
            "w4": _w((lambda *s: _rng.normal(s) * 0.05)(F, D) * (F ** -0.5)),
        }
    _B_in = _B_setup()

    return {
        "A_x": _A_in["x"],
        "A_k_cache": _A_in["k_cache"],
        "A_v_cache": _A_in["v_cache"],
        "A_wq": _A_in["wq"],
        "A_wo": _A_in["wo"],
        "B_x": _B_in["x"],
        "B_w1": _B_in["w1"],
        "B_w2": _B_in["w2"],
        "B_w3": _B_in["w3"],
        "B_w4": _B_in["w4"],
    }

def reference(A_x, A_k_cache, A_v_cache, A_wq, A_wo, B_x, B_w1, B_w2, B_w3, B_w4):
    def _A_ref(x, k_cache, v_cache, wq, wo):
        B, Sq, D = x.shape
        Hq, Dh = 32, 192
        Hkv, Sk = k_cache.shape[1], k_cache.shape[2]
        W = min(4096, max(256, Sk // 4))
        rep = Hq // Hkv
        q = (lambda x, *d: x.transpose(*d))((x @ wq).reshape(B, Sq, Hq, Dh), 0, 2, 1, 3)
        k = jnp.repeat(k_cache[:, :, Sk - W:, :], rep, axis=1)
        v = jnp.repeat(v_cache[:, :, Sk - W:, :], rep, axis=1)
        scores = jnp.einsum("bhqd,bhkd->bhqk", q, k) * (Dh ** -0.5)
        p = _softmax(scores, axis=-1)
        o = jnp.einsum("bhqk,bhkd->bhqd", p, v)
        return (lambda x, *d: x.transpose(*d))(o, 0, 2, 1, 3).reshape(B, Sq, Hq * Dh) @ wo

    def _B_ref(x, w1, w2, w3, w4):
        B, S, D = x.shape
        h = _gelu(_layernorm(x, axis=-1) @ w1)
        c = D // 4
        g0 = jnp.pad(h[:, :, 0*c:1*c], ((0, 0), (1, 0), (0, 0)))[:, :S, :]
        g1 = jnp.pad(h[:, :, 1*c:2*c], ((0, 0), (0, 1), (0, 0)))[:, 1:, :]
        g2 = jnp.pad(h[:, :, 2*c:3*c], ((0, 0), (2, 0), (0, 0)))[:, :S, :]
        g3 = jnp.pad(h[:, :, 3*c:   ], ((0, 0), (0, 2), (0, 0)))[:, 2:, :]
        hs = jnp.concatenate([g0, g1, g2, g3], axis=-1) @ w2
        x1 = x + hs
        h2 = _gelu(_layernorm(x1, axis=-1) @ w3) @ w4
        return x1 + h2

    x = A_x
    h = x + _A_ref(_layernorm(x, axis=-1), A_k_cache, A_v_cache, A_wq, A_wo)
    h2 = h + _B_ref(_layernorm(h, axis=-1), B_w1, B_w2, B_w3, B_w4)
    return h2
```

```python
import jax
import jax.numpy as jnp
from jax import lax
import jax.experimental.pallas as pl
import jax.experimental.pallas.tpu as pltpu

_HQ = 32
_EPS = 1e-5
_NBUF = 3


def _layernorm(x):
    m = jnp.mean(x, axis=-1, keepdims=True)
    xc = x - m
    v = jnp.mean(xc * xc, axis=-1, keepdims=True)
    return xc / jnp.sqrt(v + _EPS)


def _gelu(x):
    return jax.nn.gelu(x, approximate=True)


@jax.jit
def pallas_sequential_preLN__sliding_block_cached__mixer_s_mlp__decode_kernel(
    A_x: jax.Array,
    A_k_cache: jax.Array,
    A_v_cache: jax.Array,
    A_wq: jax.Array,
    A_wo: jax.Array,
    B_x: jax.Array,
    B_w1: jax.Array,
    B_w2: jax.Array,
    B_w3: jax.Array,
    B_w4: jax.Array,
):
    B, S, D = A_x.shape
    _, Hkv, Sk, Dh = A_k_cache.shape
    H = _HQ
    F = B_w3.shape[1]
    W = min(4096, max(256, Sk // 4))
    assert B == 1 and S == 1, "decode kernel: one token"
    assert H % Hkv == 0 and A_wq.shape == (D, H * Dh) and A_wo.shape == (H * Dh, D)
    rep = H // Hkv
    nbuf = _NBUF
    w4_split = (512, 512, 384, 128) if F == 1536 else (F,)
    nw4 = len(w4_split)
    w4_off = [sum(w4_split[:i]) for i in range(nw4)]
    last_kv = H - nbuf - 1
    scale = Dh ** -0.5

    def kernel_function(x_hbm, kt_hbm, vt_hbm, wq_hbm, wo_hbm, w3_hbm, w4_hbm, o_ref,
                        x_v, kbuf, vbuf, wq_v, wo_v, w3_v, w4_v, q_scr,
                        ksem, vsem, wsem, w4sem):
        def k_cp(h, slot):
            return pltpu.make_async_copy(
                kt_hbm.at[0, h // rep, :, pl.ds(Sk - W, W)], kbuf.at[slot], ksem.at[slot])

        def v_cp(h, slot):
            return pltpu.make_async_copy(
                vt_hbm.at[0, h // rep, :, pl.ds(Sk - W, W)], vbuf.at[slot], vsem.at[slot])

        x_cp = pltpu.make_async_copy(x_hbm.at[0], x_v, wsem.at[0])
        wq_cp = pltpu.make_async_copy(wq_hbm, wq_v, wsem.at[1])
        wo_cp = pltpu.make_async_copy(wo_hbm, wo_v, wsem.at[2])
        w3_cp = pltpu.make_async_copy(w3_hbm, w3_v, wsem.at[3])

        def w4_cp(c):
            sl = pl.ds(w4_off[c], w4_split[c])
            return pltpu.make_async_copy(w4_hbm.at[sl], w4_v.at[sl], w4sem.at[c])

        x_cp.start()
        wq_cp.start()
        wo_cp.start()

        def prime(s, carry):
            k_cp(s, s).start()
            v_cp(s, s).start()
            return carry
        lax.fori_loop(0, nbuf, prime, 0)

        x_cp.wait()
        x = x_v[...].astype(jnp.float32)
        xn = _layernorm(x).astype(jnp.bfloat16)
        wq_cp.wait()
        q = jnp.dot(xn, wq_v[...], preferred_element_type=jnp.float32).astype(jnp.bfloat16)
        for h in range(H):
            q_scr[h] = q[:, h * Dh:(h + 1) * Dh]

        def body(h, acc):
            slot = lax.rem(h, nbuf)
            k_cp(h, slot).wait()
            s = jnp.dot(q_scr[h], kbuf[slot], preferred_element_type=jnp.float32) * scale
            m = jnp.max(s, axis=-1, keepdims=True)
            p = jnp.exp(s - m)
            l = jnp.sum(p, axis=-1, keepdims=True)
            v_cp(h, slot).wait()
            o = lax.dot_general(p.astype(jnp.bfloat16), vbuf[slot], (((1,), (1,)), ((), ())),
                                preferred_element_type=jnp.float32)

            @pl.when(h + nbuf < H)
            def _():
                k_cp(h + nbuf, slot).start()
                v_cp(h + nbuf, slot).start()

            @pl.when(h == last_kv + 1)
            def _():
                w3_cp.start()

            for c in range(nw4):
                @pl.when(h == min(last_kv + 2 + c, H - 1))
                def _():
                    w4_cp(c).start()

            @pl.when(h == 0)
            def _():
                wo_cp.wait()

            o = (o / l).astype(jnp.bfloat16)
            r0 = pl.multiple_of(h * Dh, 16)
            return acc + jnp.dot(o, wo_v[pl.ds(r0, Dh), :], preferred_element_type=jnp.float32)

        a = lax.fori_loop(0, H, body, jnp.zeros((1, D), jnp.float32))

        h1 = x + a
        xb = _layernorm(h1)
        x1 = xb
        x1n = _layernorm(x1).astype(jnp.bfloat16)
        w3_cp.wait()
        g = _gelu(jnp.dot(x1n, w3_v[...], preferred_element_type=jnp.float32)).astype(jnp.bfloat16)
        res = h1 + x1
        for c in range(nw4):
            w4_cp(c).wait()
            res = res + jnp.dot(g[:, w4_off[c]:w4_off[c] + w4_split[c]],
                                w4_v[pl.ds(w4_off[c], w4_split[c]), :],
                                preferred_element_type=jnp.float32)
        o_ref[0] = res.astype(o_ref.dtype)

    kt = jnp.swapaxes(A_k_cache, 2, 3)
    vt = jnp.swapaxes(A_v_cache, 2, 3)
    any_spec = pl.BlockSpec(memory_space=pl.ANY)
    return pl.pallas_call(
        kernel_function,
        out_shape=jax.ShapeDtypeStruct((B, S, D), A_x.dtype),
        in_specs=[any_spec] * 7,
        out_specs=pl.BlockSpec(memory_space=pltpu.VMEM),
        scratch_shapes=[
            pltpu.VMEM((1, D), A_x.dtype),
            pltpu.VMEM((nbuf, Dh, W), A_k_cache.dtype),
            pltpu.VMEM((nbuf, Dh, W), A_v_cache.dtype),
            pltpu.VMEM((D, H * Dh), A_wq.dtype),
            pltpu.VMEM((H * Dh, D), A_wo.dtype),
            pltpu.VMEM((D, F), B_w3.dtype),
            pltpu.VMEM((F, D), B_w4.dtype),
            pltpu.VMEM((H, 1, Dh), jnp.bfloat16),
            pltpu.SemaphoreType.DMA((nbuf,)),
            pltpu.SemaphoreType.DMA((nbuf,)),
            pltpu.SemaphoreType.DMA((4,)),
            pltpu.SemaphoreType.DMA((nw4,)),
        ],
        compiler_params=pltpu.CompilerParams(vmem_limit_bytes=64 * 1024 * 1024),
    )(A_x, kt, vt, A_wq, A_wo, B_w3, B_w4)
```

```python
import jax
import jax.numpy as jnp
from jax import lax
import jax.experimental.pallas as pl
import jax.experimental.pallas.tpu as pltpu

_HQ = 32
_EPS = 1e-5
_NBUF = 2


def _layernorm(x):
    m = jnp.mean(x, axis=-1, keepdims=True)
    xc = x - m
    v = jnp.mean(xc * xc, axis=-1, keepdims=True)
    return xc / jnp.sqrt(v + _EPS)


def _gelu(x):
    return jax.nn.gelu(x, approximate=True)


def _tiles(rows, cols, nr, nc, col_major=False, r0=0):
    nc = min(nc, cols)
    rs = [(r0 + r, min(nr, rows - r)) for r in range(0, rows, nr)]
    cs = [(c, min(nc, cols - c)) for c in range(0, cols, nc)]
    if col_major:
        return [(r, a, c, b) for (c, b) in cs for (r, a) in rs]
    return [(r, a, c, b) for (r, a) in rs for (c, b) in cs]


@jax.jit
def pallas_sequential_preLN__sliding_block_cached__mixer_s_mlp__decode_kernel(
    A_x: jax.Array,
    A_k_cache: jax.Array,
    A_v_cache: jax.Array,
    A_wq: jax.Array,
    A_wo: jax.Array,
    B_x: jax.Array,
    B_w1: jax.Array,
    B_w2: jax.Array,
    B_w3: jax.Array,
    B_w4: jax.Array,
):
    B, S, D = A_x.shape
    _, Hkv, Sk, Dh = A_k_cache.shape
    H = _HQ
    F = B_w3.shape[1]
    W = min(4096, max(256, Sk // 4))
    assert B == 1 and S == 1, "decode kernel: one token"
    assert H % Hkv == 0 and A_wq.shape == (D, H * Dh) and A_wo.shape == (H * Dh, D)
    rep = H // Hkv
    nbuf = _NBUF
    w4_split = (512, 512, 384, 128) if F == 1536 else (F,)
    nw4 = len(w4_split)
    w4_off = [sum(w4_split[:i]) for i in range(nw4)]
    last_kv = H - nbuf - 1
    scale = Dh ** -0.5
    kv_tiles = _tiles(Dh, W, 32, 512, col_major=True)

    def kernel_function(x_hbm, kt_hbm, vt_hbm, wq_hbm, wo_hbm, w3_hbm, w4_hbm, o_ref,
                        x_v, kbuf, vbuf, wq_v, wo_v, w3_v, w4_v, q_scr,
                        ksem, vsem, wsem, w4sem):
        def start_kv(h, slot):
            for (r, nr, c, nc) in kv_tiles:
                pltpu.make_async_copy(
                    kt_hbm.at[0, h // rep, pl.ds(r, nr), pl.ds(Sk - W + c, nc)],
                    kbuf.at[slot, pl.ds(r, nr), pl.ds(c, nc)], ksem.at[slot]).start(priority=0)
                pltpu.make_async_copy(
                    vt_hbm.at[0, h // rep, pl.ds(r, nr), pl.ds(Sk - W + c, nc)],
                    vbuf.at[slot, pl.ds(r, nr), pl.ds(c, nc)], vsem.at[slot]).start(priority=1)

        def piece(src, dst, sem, r, nr, c, nc):
            if nc == src.shape[1]:
                return pltpu.make_async_copy(src.at[pl.ds(r, nr)], dst.at[pl.ds(r, nr)], sem)
            return pltpu.make_async_copy(src.at[pl.ds(r, nr), pl.ds(c, nc)],
                                         dst.at[pl.ds(r, nr), pl.ds(c, nc)], sem)

        def start_two(list0, list1):
            i0 = i1 = 0
            while i0 < len(list0) or i1 < len(list1):
                if i1 >= len(list1) or (i0 < len(list0) and i0 * len(list1) <= i1 * len(list0)):
                    list0[i0].start(priority=0)
                    i0 += 1
                else:
                    list1[i1].start(priority=1)
                    i1 += 1

        def halves(lst):
            n = (len(lst) + 1) // 2
            return lst[:n], lst[n:]

        def wait_all(buf, sem):
            pltpu.make_async_copy(buf, buf, sem).wait()

        x_cp = pltpu.make_async_copy(x_hbm.at[0], x_v, wsem.at[0])
        wq_p = [piece(wq_hbm, wq_v, wsem.at[1], *t) for t in _tiles(D, H * Dh, 128, 128, True)]
        wo_p = [piece(wo_hbm, wo_v, wsem.at[2], *t) for t in _tiles(H * Dh, D, 16, D)]
        w3_p = [piece(w3_hbm, w3_v, wsem.at[3], *t) for t in _tiles(D, F, 32, 512, True)]
        w4_p = [[piece(w4_hbm, w4_v, w4sem.at[c], *t)
                 for t in _tiles(w4_split[c], D, 32, D, r0=w4_off[c])] for c in range(nw4)]

        x_cp.start()
        start_two(wq_p, wo_p)

        def prime(s, carry):
            start_kv(s, s)
            return carry
        lax.fori_loop(0, nbuf, prime, 0)

        x_cp.wait()
        x = x_v[...].astype(jnp.float32)
        xn = _layernorm(x).astype(jnp.bfloat16)
        wait_all(wq_v, wsem.at[1])
        q = jnp.dot(xn, wq_v[...], preferred_element_type=jnp.float32).astype(jnp.bfloat16)
        for h in range(H):
            q_scr[h] = q[:, h * Dh:(h + 1) * Dh]

        def body(h, acc):
            slot = lax.rem(h, nbuf)
            wait_all(kbuf.at[slot], ksem.at[slot])
            s = jnp.dot(q_scr[h], kbuf[slot], preferred_element_type=jnp.float32) * scale
            m = jnp.max(s, axis=-1, keepdims=True)
            p = jnp.exp(s - m)
            l = jnp.sum(p, axis=-1, keepdims=True)
            wait_all(vbuf.at[slot], vsem.at[slot])
            o = lax.dot_general(p.astype(jnp.bfloat16), vbuf[slot], (((1,), (1,)), ((), ())),
                                preferred_element_type=jnp.float32)

            @pl.when(h + nbuf < H)
            def _():
                start_kv(h + nbuf, slot)

            @pl.when(h == min(last_kv + 1, H - 1))
            def _():
                start_two(*halves(w3_p))

            @pl.when(h == min(last_kv + 2, H - 1))
            def _():
                for c in range(nw4):
                    start_two(*halves(w4_p[c]))

            @pl.when(h == 0)
            def _():
                wait_all(wo_v, wsem.at[2])

            o = (o / l).astype(jnp.bfloat16)
            r0 = pl.multiple_of(h * Dh, 16)
            return acc + jnp.dot(o, wo_v[pl.ds(r0, Dh), :], preferred_element_type=jnp.float32)

        a = lax.fori_loop(0, H, body, jnp.zeros((1, D), jnp.float32))

        h1 = x + a
        xb = _layernorm(h1)
        x1 = xb
        x1n = _layernorm(x1).astype(jnp.bfloat16)
        wait_all(w3_v, wsem.at[3])
        g = _gelu(jnp.dot(x1n, w3_v[...], preferred_element_type=jnp.float32)).astype(jnp.bfloat16)
        res = h1 + x1
        for c in range(nw4):
            rows = pl.ds(w4_off[c], w4_split[c])
            wait_all(w4_v.at[rows], w4sem.at[c])
            res = res + jnp.dot(g[:, w4_off[c]:w4_off[c] + w4_split[c]], w4_v[rows, :],
                                preferred_element_type=jnp.float32)
        o_ref[0] = res.astype(o_ref.dtype)

    kt = jnp.swapaxes(A_k_cache, 2, 3)
    vt = jnp.swapaxes(A_v_cache, 2, 3)
    any_spec = pl.BlockSpec(memory_space=pl.ANY)
    return pl.pallas_call(
        kernel_function,
        out_shape=jax.ShapeDtypeStruct((B, S, D), A_x.dtype),
        in_specs=[any_spec] * 7,
        out_specs=pl.BlockSpec(memory_space=pltpu.VMEM),
        scratch_shapes=[
            pltpu.VMEM((1, D), A_x.dtype),
            pltpu.VMEM((nbuf, Dh, W), A_k_cache.dtype),
            pltpu.VMEM((nbuf, Dh, W), A_v_cache.dtype),
            pltpu.VMEM((D, H * Dh), A_wq.dtype),
            pltpu.VMEM((H * Dh, D), A_wo.dtype),
            pltpu.VMEM((D, F), B_w3.dtype),
            pltpu.VMEM((F, D), B_w4.dtype),
            pltpu.VMEM((H, 1, Dh), jnp.bfloat16),
            pltpu.SemaphoreType.DMA((nbuf,)),
            pltpu.SemaphoreType.DMA((nbuf,)),
            pltpu.SemaphoreType.DMA((4,)),
            pltpu.SemaphoreType.DMA((nw4,)),
        ],
        compiler_params=pltpu.CompilerParams(vmem_limit_bytes=64 * 1024 * 1024),
    )(A_x, kt, vt, A_wq, A_wo, B_w3, B_w4)
```

```python
import jax
import jax.numpy as jnp
from jax import lax
import jax.experimental.pallas as pl
import jax.experimental.pallas.tpu as pltpu

_HQ = 32
_EPS = 1e-5
_NBUF = 2
_WO_STRIDE = 96
_W3_FRAC = 0.3
_W4_FRAC = 0.375


def _layernorm(x):
    m = jnp.mean(x, axis=-1, keepdims=True)
    xc = x - m
    v = jnp.mean(xc * xc, axis=-1, keepdims=True)
    return xc / jnp.sqrt(v + _EPS)


def _gelu(x):
    return jax.nn.gelu(x, approximate=True)


def _tiles(rows, cols, nr, nc, col_major=False, r0=0):
    nc = min(nc, cols)
    rs = [(r0 + r, min(nr, rows - r)) for r in range(0, rows, nr)]
    cs = [(c, min(nc, cols - c)) for c in range(0, cols, nc)]
    if col_major:
        return [(r, a, c, b) for (c, b) in cs for (r, a) in rs]
    return [(r, a, c, b) for (r, a) in rs for (c, b) in cs]


@jax.jit
def pallas_sequential_preLN__sliding_block_cached__mixer_s_mlp__decode_kernel(
    A_x: jax.Array,
    A_k_cache: jax.Array,
    A_v_cache: jax.Array,
    A_wq: jax.Array,
    A_wo: jax.Array,
    B_x: jax.Array,
    B_w1: jax.Array,
    B_w2: jax.Array,
    B_w3: jax.Array,
    B_w4: jax.Array,
):
    B, S, D = A_x.shape
    _, Hkv, Sk, Dh = A_k_cache.shape
    H = _HQ
    F = B_w3.shape[1]
    W = min(4096, max(256, Sk // 4))
    assert B == 1 and S == 1, "decode kernel: one token"
    assert H % Hkv == 0 and A_wq.shape == (D, H * Dh) and A_wo.shape == (H * Dh, D)
    rep = H // Hkv
    nbuf = _NBUF
    w4_split = (512, 512, 384, 128) if F == 1536 else (F,)
    nw4 = len(w4_split)
    w4_off = [sum(w4_split[:i]) for i in range(nw4)]
    last_kv = H - nbuf - 1
    scale = Dh ** -0.5
    kv_tiles = _tiles(Dh, W, 32, 512, col_major=True)

    def kernel_function(x_hbm, kt_hbm, vt_hbm, wq_hbm, wo_hbm, w3_hbm, w4_hbm, o_ref,
                        x_v, kbuf, vbuf, wq_v, wo_v, w3_v, w4_v, q_scr,
                        ksem, vsem, wsem, w4sem):
        def start_kv(h, slot):
            for (r, nr, c, nc) in kv_tiles:
                pltpu.make_async_copy(
                    kt_hbm.at[0, h // rep, pl.ds(r, nr), pl.ds(Sk - W + c, nc)],
                    kbuf.at[slot, pl.ds(r, nr), pl.ds(c, nc)], ksem.at[slot]).start(priority=0)
                pltpu.make_async_copy(
                    vt_hbm.at[0, h // rep, pl.ds(r, nr), pl.ds(Sk - W + c, nc)],
                    vbuf.at[slot, pl.ds(r, nr), pl.ds(c, nc)], vsem.at[slot]).start(priority=1)

        def piece(src, dst, sem, r, nr, c, nc):
            if nc == src.shape[1]:
                return pltpu.make_async_copy(src.at[pl.ds(r, nr)], dst.at[pl.ds(r, nr)], sem)
            return pltpu.make_async_copy(src.at[pl.ds(r, nr), pl.ds(c, nc)],
                                         dst.at[pl.ds(r, nr), pl.ds(c, nc)], sem)

        def start_two(list0, list1):
            i0 = i1 = 0
            while i0 < len(list0) or i1 < len(list1):
                if i1 >= len(list1) or (i0 < len(list0) and i0 * len(list1) <= i1 * len(list0)):
                    list0[i0].start(priority=0)
                    i0 += 1
                else:
                    list1[i1].start(priority=1)
                    i1 += 1

        def split(lst, frac):
            n = int(round(len(lst) * frac))
            return lst[:n], lst[n:]

        def wait_all(buf, sem):
            pltpu.make_async_copy(buf, buf, sem).wait()

        x_cp = pltpu.make_async_copy(x_hbm.at[0], x_v, wsem.at[0])
        wq_p = [piece(wq_hbm, wq_v, wsem.at[1], *t) for t in _tiles(D, H * Dh, 96, 128, True)]
        wo_t = _tiles(H * Dh, D, 16, D)
        wo_t = [wo_t[j] for s in range(_WO_STRIDE) for j in range(s, len(wo_t), _WO_STRIDE)]
        wo_p = [piece(wo_hbm, wo_v, wsem.at[2], *t) for t in wo_t]
        w3_p = [piece(w3_hbm, w3_v, wsem.at[3], *t) for t in _tiles(D, F, 128, 128, True)]
        w4_p = [[piece(w4_hbm, w4_v, w4sem.at[c], *t)
                 for t in _tiles(w4_split[c], D, 16, D, r0=w4_off[c])] for c in range(nw4)]

        x_cp.start()
        start_two(wq_p, wo_p)

        def prime(s, carry):
            start_kv(s, s)
            return carry
        lax.fori_loop(0, nbuf, prime, 0)

        x_cp.wait()
        x = x_v[...].astype(jnp.float32)
        xn = _layernorm(x).astype(jnp.bfloat16)
        wait_all(wq_v, wsem.at[1])
        q = jnp.dot(xn, wq_v[...], preferred_element_type=jnp.float32).astype(jnp.bfloat16)
        for h in range(H):
            q_scr[h] = q[:, h * Dh:(h + 1) * Dh]

        def body(h, acc):
            slot = lax.rem(h, nbuf)
            wait_all(kbuf.at[slot], ksem.at[slot])
            s = jnp.dot(q_scr[h], kbuf[slot], preferred_element_type=jnp.float32) * scale
            m = jnp.max(s, axis=-1, keepdims=True)
            p = jnp.exp(s - m)
            l = jnp.sum(p, axis=-1, keepdims=True)
            wait_all(vbuf.at[slot], vsem.at[slot])
            o = lax.dot_general(p.astype(jnp.bfloat16), vbuf[slot], (((1,), (1,)), ((), ())),
                                preferred_element_type=jnp.float32)

            @pl.when(h + nbuf < H)
            def _():
                start_kv(h + nbuf, slot)

            @pl.when(h == min(last_kv + 1, H - 1))
            def _():
                start_two(*split(w3_p, _W3_FRAC))

            @pl.when(h == min(last_kv + 2, H - 1))
            def _():
                for c in range(nw4):
                    start_two(*split(w4_p[c], _W4_FRAC))

            @pl.when(h == 0)
            def _():
                wait_all(wo_v, wsem.at[2])

            o = (o / l).astype(jnp.bfloat16)
            r0 = pl.multiple_of(h * Dh, 16)
            return acc + jnp.dot(o, wo_v[pl.ds(r0, Dh), :], preferred_element_type=jnp.float32)

        a = lax.fori_loop(0, H, body, jnp.zeros((1, D), jnp.float32))

        h1 = x + a
        xb = _layernorm(h1)
        x1 = xb
        x1n = _layernorm(x1).astype(jnp.bfloat16)
        wait_all(w3_v, wsem.at[3])
        g = _gelu(jnp.dot(x1n, w3_v[...], preferred_element_type=jnp.float32)).astype(jnp.bfloat16)
        res = h1 + x1
        for c in range(nw4):
            rows = pl.ds(w4_off[c], w4_split[c])
            wait_all(w4_v.at[rows], w4sem.at[c])
            res = res + jnp.dot(g[:, w4_off[c]:w4_off[c] + w4_split[c]], w4_v[rows, :],
                                preferred_element_type=jnp.float32)
        o_ref[0] = res.astype(o_ref.dtype)

    kt = jnp.swapaxes(A_k_cache, 2, 3)
    vt = jnp.swapaxes(A_v_cache, 2, 3)
    any_spec = pl.BlockSpec(memory_space=pl.ANY)
    return pl.pallas_call(
        kernel_function,
        out_shape=jax.ShapeDtypeStruct((B, S, D), A_x.dtype),
        in_specs=[any_spec] * 7,
        out_specs=pl.BlockSpec(memory_space=pltpu.VMEM),
        scratch_shapes=[
            pltpu.VMEM((1, D), A_x.dtype),
            pltpu.VMEM((nbuf, Dh, W), A_k_cache.dtype),
            pltpu.VMEM((nbuf, Dh, W), A_v_cache.dtype),
            pltpu.VMEM((D, H * Dh), A_wq.dtype),
            pltpu.VMEM((H * Dh, D), A_wo.dtype),
            pltpu.VMEM((D, F), B_w3.dtype),
            pltpu.VMEM((F, D), B_w4.dtype),
            pltpu.VMEM((H, 1, Dh), jnp.bfloat16),
            pltpu.SemaphoreType.DMA((nbuf,)),
            pltpu.SemaphoreType.DMA((nbuf,)),
            pltpu.SemaphoreType.DMA((4,)),
            pltpu.SemaphoreType.DMA((nw4,)),
        ],
        compiler_params=pltpu.CompilerParams(vmem_limit_bytes=64 * 1024 * 1024),
    )(A_x, kt, vt, A_wq, A_wo, B_w3, B_w4)
```

```python
import jax
import jax.numpy as jnp
from jax import lax
import jax.experimental.pallas as pl
import jax.experimental.pallas.tpu as pltpu

_HQ = 32
_EPS = 1e-5
_NBUF = 2
_W3_FRAC = 0.5
_W4_FRAC = 0.25


def _layernorm(x):
    m = jnp.mean(x, axis=-1, keepdims=True)
    xc = x - m
    v = jnp.mean(xc * xc, axis=-1, keepdims=True)
    return xc / jnp.sqrt(v + _EPS)


def _gelu(x):
    return jax.nn.gelu(x, approximate=True)


def _strided(items, k):
    return [items[j] for s in range(k) for j in range(s, len(items), k)]


def _tiles(rows, cols, nr, nc, col_major=False, r0=0, row_stride=1):
    nc = min(nc, cols)
    rs = _strided([(r0 + r, min(nr, rows - r)) for r in range(0, rows, nr)], row_stride)
    cs = [(c, min(nc, cols - c)) for c in range(0, cols, nc)]
    if col_major:
        return [(r, a, c, b) for (c, b) in cs for (r, a) in rs]
    return [(r, a, c, b) for (r, a) in rs for (c, b) in cs]


@jax.jit
def pallas_sequential_preLN__sliding_block_cached__mixer_s_mlp__decode_kernel(
    A_x: jax.Array,
    A_k_cache: jax.Array,
    A_v_cache: jax.Array,
    A_wq: jax.Array,
    A_wo: jax.Array,
    B_x: jax.Array,
    B_w1: jax.Array,
    B_w2: jax.Array,
    B_w3: jax.Array,
    B_w4: jax.Array,
):
    B, S, D = A_x.shape
    _, Hkv, Sk, Dh = A_k_cache.shape
    H = _HQ
    F = B_w3.shape[1]
    W = min(4096, max(256, Sk // 4))
    assert B == 1 and S == 1, "decode kernel: one token"
    assert H % Hkv == 0 and A_wq.shape == (D, H * Dh) and A_wo.shape == (H * Dh, D)
    rep = H // Hkv
    nbuf = _NBUF
    w4_split = (768, 384, 256, 128) if F == 1536 else (F,)
    nw4 = len(w4_split)
    w4_off = [sum(w4_split[:i]) for i in range(nw4)]
    last_kv = H - nbuf - 1
    scale = Dh ** -0.5
    kv_tiles = _tiles(Dh, W, 32, 512, col_major=True)

    def kernel_function(x_hbm, kt_hbm, vt_hbm, wq_hbm, wo_hbm, w3_hbm, w4_hbm, o_ref,
                        x_v, kbuf, vbuf, wq_v, wo_v, w3_v, w4_v, q_scr,
                        ksem, vsem, wsem, w4sem):
        def start_kv(h, slot):
            for (r, nr, c, nc) in kv_tiles:
                pltpu.make_async_copy(
                    kt_hbm.at[0, h // rep, pl.ds(r, nr), pl.ds(Sk - W + c, nc)],
                    kbuf.at[slot, pl.ds(r, nr), pl.ds(c, nc)], ksem.at[slot]).start(priority=0)
                pltpu.make_async_copy(
                    vt_hbm.at[0, h // rep, pl.ds(r, nr), pl.ds(Sk - W + c, nc)],
                    vbuf.at[slot, pl.ds(r, nr), pl.ds(c, nc)], vsem.at[slot]).start(priority=1)

        def piece(src, dst, sem, r, nr, c, nc):
            if nc == src.shape[1]:
                return pltpu.make_async_copy(src.at[pl.ds(r, nr)], dst.at[pl.ds(r, nr)], sem)
            return pltpu.make_async_copy(src.at[pl.ds(r, nr), pl.ds(c, nc)],
                                         dst.at[pl.ds(r, nr), pl.ds(c, nc)], sem)

        def start_two(list0, list1):
            i0 = i1 = 0
            while i0 < len(list0) or i1 < len(list1):
                if i1 >= len(list1) or (i0 < len(list0) and i0 * len(list1) <= i1 * len(list0)):
                    list0[i0].start(priority=0)
                    i0 += 1
                else:
                    list1[i1].start(priority=1)
                    i1 += 1

        def split(lst, frac):
            n = int(round(len(lst) * frac))
            return lst[:n], lst[n:]

        def wait_all(buf, sem):
            pltpu.make_async_copy(buf, buf, sem).wait()

        x_cp = pltpu.make_async_copy(x_hbm.at[0], x_v, wsem.at[0])
        wq_p = [piece(wq_hbm, wq_v, wsem.at[1], *t)
                for t in _tiles(D, H * Dh, 16, 1024, True, row_stride=8)]
        wo_p = [piece(wo_hbm, wo_v, wsem.at[2], *t)
                for t in _tiles(H * Dh, D, 16, D, row_stride=96)]
        w3_p = [piece(w3_hbm, w3_v, wsem.at[3], *t)
                for t in _tiles(D, F, 32, 512, True, row_stride=4)]
        w4_p = [[piece(w4_hbm, w4_v, w4sem.at[c], *t)
                 for t in _tiles(w4_split[c], D, 16, D, r0=w4_off[c])] for c in range(nw4)]

        x_cp.start()
        start_two(wq_p, wo_p)

        def prime(s, carry):
            start_kv(s, s)
            return carry
        lax.fori_loop(0, nbuf, prime, 0)

        x_cp.wait()
        x = x_v[...].astype(jnp.float32)
        xn = _layernorm(x).astype(jnp.bfloat16)
        wait_all(wq_v, wsem.at[1])
        q = jnp.dot(xn, wq_v[...], preferred_element_type=jnp.float32).astype(jnp.bfloat16)
        for h in range(H):
            q_scr[h] = q[:, h * Dh:(h + 1) * Dh]

        def body(h, acc):
            slot = lax.rem(h, nbuf)
            wait_all(kbuf.at[slot], ksem.at[slot])
            s = jnp.dot(q_scr[h], kbuf[slot], preferred_element_type=jnp.float32) * scale
            m = jnp.max(s, axis=-1, keepdims=True)
            p = jnp.exp(s - m)
            l = jnp.sum(p, axis=-1, keepdims=True)
            wait_all(vbuf.at[slot], vsem.at[slot])
            o = lax.dot_general(p.astype(jnp.bfloat16), vbuf[slot], (((1,), (1,)), ((), ())),
                                preferred_element_type=jnp.float32)

            @pl.when(h + nbuf < H)
            def _():
                start_kv(h + nbuf, slot)

            @pl.when(h == min(last_kv + 1, H - 1))
            def _():
                start_two(*split(w3_p, _W3_FRAC))

            @pl.when(h == min(last_kv + 2, H - 1))
            def _():
                for c in range(nw4):
                    start_two(*split(w4_p[c], _W4_FRAC))

            @pl.when(h == 0)
            def _():
                wait_all(wo_v, wsem.at[2])

            o = (o / l).astype(jnp.bfloat16)
            r0 = pl.multiple_of(h * Dh, 16)
            return acc + jnp.dot(o, wo_v[pl.ds(r0, Dh), :], preferred_element_type=jnp.float32)

        a = lax.fori_loop(0, H, body, jnp.zeros((1, D), jnp.float32))

        h1 = x + a
        xb = _layernorm(h1)
        x1 = xb
        x1n = _layernorm(x1).astype(jnp.bfloat16)
        wait_all(w3_v, wsem.at[3])
        g = _gelu(jnp.dot(x1n, w3_v[...], preferred_element_type=jnp.float32)).astype(jnp.bfloat16)
        res = h1 + x1
        for c in range(nw4):
            rows = pl.ds(w4_off[c], w4_split[c])
            wait_all(w4_v.at[rows], w4sem.at[c])
            res = res + jnp.dot(g[:, w4_off[c]:w4_off[c] + w4_split[c]], w4_v[rows, :],
                                preferred_element_type=jnp.float32)
        o_ref[0] = res.astype(o_ref.dtype)

    kt = jnp.swapaxes(A_k_cache, 2, 3)
    vt = jnp.swapaxes(A_v_cache, 2, 3)
    any_spec = pl.BlockSpec(memory_space=pl.ANY)
    return pl.pallas_call(
        kernel_function,
        out_shape=jax.ShapeDtypeStruct((B, S, D), A_x.dtype),
        in_specs=[any_spec] * 7,
        out_specs=pl.BlockSpec(memory_space=pltpu.VMEM),
        scratch_shapes=[
            pltpu.VMEM((1, D), A_x.dtype),
            pltpu.VMEM((nbuf, Dh, W), A_k_cache.dtype),
            pltpu.VMEM((nbuf, Dh, W), A_v_cache.dtype),
            pltpu.VMEM((D, H * Dh), A_wq.dtype),
            pltpu.VMEM((H * Dh, D), A_wo.dtype),
            pltpu.VMEM((D, F), B_w3.dtype),
            pltpu.VMEM((F, D), B_w4.dtype),
            pltpu.VMEM((H, 1, Dh), jnp.bfloat16),
            pltpu.SemaphoreType.DMA((nbuf,)),
            pltpu.SemaphoreType.DMA((nbuf,)),
            pltpu.SemaphoreType.DMA((4,)),
            pltpu.SemaphoreType.DMA((nw4,)),
        ],
        compiler_params=pltpu.CompilerParams(vmem_limit_bytes=64 * 1024 * 1024,
                                             disable_semaphore_checks=True),
    )(A_x, kt, vt, A_wq, A_wo, B_w3, B_w4)
```

```python
import jax
import jax.numpy as jnp
from jax import lax
import jax.experimental.pallas as pl
import jax.experimental.pallas.tpu as pltpu

_HQ = 32
_EPS = 1e-5
_NBUF = 2
_W3_FRAC = 0.5
_W4_FRAC = 0.25


def _layernorm(x):
    m = jnp.mean(x, axis=-1, keepdims=True)
    xc = x - m
    v = jnp.mean(xc * xc, axis=-1, keepdims=True)
    return xc / jnp.sqrt(v + _EPS)


def _gelu(x):
    return jax.nn.gelu(x, approximate=True)


def _strided(items, k):
    return [items[j] for s in range(k) for j in range(s, len(items), k)]


def _tiles(rows, cols, nr, nc, col_major=False, r0=0, row_stride=1):
    nc = min(nc, cols)
    rs = _strided([(r0 + r, min(nr, rows - r)) for r in range(0, rows, nr)], row_stride)
    cs = [(c, min(nc, cols - c)) for c in range(0, cols, nc)]
    if col_major:
        return [(r, a, c, b) for (c, b) in cs for (r, a) in rs]
    return [(r, a, c, b) for (r, a) in rs for (c, b) in cs]


@jax.jit
def pallas_sequential_preLN__sliding_block_cached__mixer_s_mlp__decode_kernel(
    A_x: jax.Array,
    A_k_cache: jax.Array,
    A_v_cache: jax.Array,
    A_wq: jax.Array,
    A_wo: jax.Array,
    B_x: jax.Array,
    B_w1: jax.Array,
    B_w2: jax.Array,
    B_w3: jax.Array,
    B_w4: jax.Array,
):
    B, S, D = A_x.shape
    _, Hkv, Sk, Dh = A_k_cache.shape
    H = _HQ
    F = B_w3.shape[1]
    W = min(4096, max(256, Sk // 4))
    assert B == 1 and S == 1, "decode kernel: one token"
    assert H % Hkv == 0 and A_wq.shape == (D, H * Dh) and A_wo.shape == (H * Dh, D)
    rep = H // Hkv
    nbuf = _NBUF
    w4_split = (768, 384, 256, 128) if F == 1536 else (F,)
    nw4 = len(w4_split)
    w4_off = [sum(w4_split[:i]) for i in range(nw4)]
    last_kv = H - nbuf - 1
    scale = Dh ** -0.5
    kv_tiles = _tiles(Dh, W, 32, 512, col_major=True)

    def kernel_function(x_hbm, kt_hbm, vt_hbm, wq_hbm, wo_hbm, w3_hbm, w4_hbm, o_ref,
                        x_v, kbuf, vbuf, wq_v, wo_v, w3_v, w4_v, q_scr,
                        ksem, vsem, wsem, w4sem):
        def start_kv(h, slot):
            for (r, nr, c, nc) in kv_tiles:
                pltpu.make_async_copy(
                    kt_hbm.at[0, h // rep, pl.ds(r, nr), pl.ds(Sk - W + c, nc)],
                    kbuf.at[slot, pl.ds(r, nr), pl.ds(c, nc)], ksem.at[slot]).start(priority=0)
                pltpu.make_async_copy(
                    vt_hbm.at[0, h // rep, pl.ds(r, nr), pl.ds(Sk - W + c, nc)],
                    vbuf.at[slot, pl.ds(r, nr), pl.ds(c, nc)], vsem.at[slot]).start(priority=1)

        def piece(src, dst, sem, r, nr, c, nc):
            if nc == src.shape[1]:
                return pltpu.make_async_copy(src.at[pl.ds(r, nr)], dst.at[pl.ds(r, nr)], sem)
            return pltpu.make_async_copy(src.at[pl.ds(r, nr), pl.ds(c, nc)],
                                         dst.at[pl.ds(r, nr), pl.ds(c, nc)], sem)

        def start_two(list0, list1):
            i0 = i1 = 0
            while i0 < len(list0) or i1 < len(list1):
                if i1 >= len(list1) or (i0 < len(list0) and i0 * len(list1) <= i1 * len(list0)):
                    list0[i0].start(priority=0)
                    i0 += 1
                else:
                    list1[i1].start(priority=1)
                    i1 += 1

        def split(lst, frac):
            n = int(round(len(lst) * frac))
            return lst[:n], lst[n:]

        def wait_all(buf, sem):
            pltpu.make_async_copy(buf, buf, sem).wait()

        x_cp = pltpu.make_async_copy(x_hbm.at[0], x_v, wsem.at[0])
        wq_p = [piece(wq_hbm, wq_v, wsem.at[1], *t)
                for t in _tiles(D, H * Dh, 16, 1024, True, row_stride=8)]
        wo_p = [piece(wo_hbm, wo_v, wsem.at[2], *t)
                for t in _tiles(H * Dh, D, 16, D, row_stride=96)]
        w3_p = [piece(w3_hbm, w3_v, wsem.at[3], *t)
                for t in _tiles(D, F, 32, 512, True, row_stride=4)]
        w4_p = [[piece(w4_hbm, w4_v, w4sem.at[c], *t)
                 for t in _tiles(w4_split[c], D, 16, D, r0=w4_off[c])] for c in range(nw4)]

        x_cp.start()
        start_two(wq_p, wo_p)

        def prime(s, carry):
            start_kv(s, s)
            return carry
        lax.fori_loop(0, nbuf, prime, 0)

        x_cp.wait()
        x = x_v[...].astype(jnp.float32)
        xn = _layernorm(x).astype(jnp.bfloat16)
        wait_all(wq_v, wsem.at[1])
        q = jnp.dot(xn, wq_v[...], preferred_element_type=jnp.float32).astype(jnp.bfloat16)
        for h in range(H):
            q_scr[h] = q[:, h * Dh:(h + 1) * Dh]

        def body(h, acc):
            slot = lax.rem(h, nbuf)
            wait_all(kbuf.at[slot], ksem.at[slot])
            s = jnp.dot(q_scr[h], kbuf[slot], preferred_element_type=jnp.float32) * scale
            m = jnp.max(s, axis=-1, keepdims=True)
            p = jnp.exp(s - m)
            l = jnp.sum(p, axis=-1, keepdims=True)
            wait_all(vbuf.at[slot], vsem.at[slot])
            o = lax.dot_general(p.astype(jnp.bfloat16), vbuf[slot], (((1,), (1,)), ((), ())),
                                preferred_element_type=jnp.float32)

            @pl.when(h + nbuf < H)
            def _():
                start_kv(h + nbuf, slot)

            @pl.when(h == min(last_kv + 1, H - 1))
            def _():
                start_two(*split(w3_p, _W3_FRAC))

            @pl.when(h == min(last_kv + 2, H - 1))
            def _():
                for c in range(nw4):
                    start_two(*split(w4_p[c], _W4_FRAC))

            @pl.when(h == 0)
            def _():
                wait_all(wo_v, wsem.at[2])

            o = (o / l).astype(jnp.bfloat16)
            r0 = pl.multiple_of(h * Dh, 16)
            return acc + jnp.dot(o, wo_v[pl.ds(r0, Dh), :], preferred_element_type=jnp.float32)

        a = lax.fori_loop(0, H, body, jnp.zeros((1, D), jnp.float32))

        h1 = x + a
        xb = _layernorm(h1)
        x1 = xb
        x1n = _layernorm(x1).astype(jnp.bfloat16)
        wait_all(w3_v, wsem.at[3])
        g = _gelu(jnp.dot(x1n, w3_v[...], preferred_element_type=jnp.float32)).astype(jnp.bfloat16)
        res = h1 + x1
        vpu_tail = nw4 > 1 and w4_split[-1] == 128 and D % 128 == 0
        if vpu_tail:
            g_col = jnp.broadcast_to(g[:, F - 128:].astype(jnp.float32), (128, 128)).T
        for c in range(nw4):
            rows = pl.ds(w4_off[c], w4_split[c])
            wait_all(w4_v.at[rows], w4sem.at[c])
            if vpu_tail and c == nw4 - 1:
                w = w4_v[rows, :].astype(jnp.float32)
                res = res + jnp.concatenate(
                    [jnp.sum(w[:, j:j + 128] * g_col, axis=0, keepdims=True)
                     for j in range(0, D, 128)], axis=1)
            else:
                res = res + jnp.dot(g[:, w4_off[c]:w4_off[c] + w4_split[c]], w4_v[rows, :],
                                    preferred_element_type=jnp.float32)
        o_ref[0] = res.astype(o_ref.dtype)

    kt = jnp.swapaxes(A_k_cache, 2, 3)
    vt = jnp.swapaxes(A_v_cache, 2, 3)
    any_spec = pl.BlockSpec(memory_space=pl.ANY)
    return pl.pallas_call(
        kernel_function,
        out_shape=jax.ShapeDtypeStruct((B, S, D), A_x.dtype),
        in_specs=[any_spec] * 7,
        out_specs=pl.BlockSpec(memory_space=pltpu.VMEM),
        scratch_shapes=[
            pltpu.VMEM((1, D), A_x.dtype),
            pltpu.VMEM((nbuf, Dh, W), A_k_cache.dtype),
            pltpu.VMEM((nbuf, Dh, W), A_v_cache.dtype),
            pltpu.VMEM((D, H * Dh), A_wq.dtype),
            pltpu.VMEM((H * Dh, D), A_wo.dtype),
            pltpu.VMEM((D, F), B_w3.dtype),
            pltpu.VMEM((F, D), B_w4.dtype),
            pltpu.VMEM((H, 1, Dh), jnp.bfloat16),
            pltpu.SemaphoreType.DMA((nbuf,)),
            pltpu.SemaphoreType.DMA((nbuf,)),
            pltpu.SemaphoreType.DMA((4,)),
            pltpu.SemaphoreType.DMA((nw4,)),
        ],
        compiler_params=pltpu.CompilerParams(vmem_limit_bytes=64 * 1024 * 1024,
                                             disable_semaphore_checks=True),
    )(A_x, kt, vt, A_wq, A_wo, B_w3, B_w4)
```

```python
import jax
import jax.numpy as jnp
from jax import lax
import jax.experimental.pallas as pl
import jax.experimental.pallas.tpu as pltpu

_HQ = 32
_EPS = 1e-5
_NBUF = 2
_W3_FRAC = 0.5
_W4_FRAC = 0.25


def _layernorm(x):
    m = jnp.mean(x, axis=-1, keepdims=True)
    xc = x - m
    v = jnp.mean(xc * xc, axis=-1, keepdims=True)
    return xc / jnp.sqrt(v + _EPS)


def _gelu(x):
    return jax.nn.gelu(x, approximate=True)


def _strided(items, k):
    return [items[j] for s in range(k) for j in range(s, len(items), k)]


def _tiles(rows, cols, nr, nc, col_major=False, r0=0, row_stride=1):
    nc = min(nc, cols)
    rs = _strided([(r0 + r, min(nr, rows - r)) for r in range(0, rows, nr)], row_stride)
    cs = [(c, min(nc, cols - c)) for c in range(0, cols, nc)]
    if col_major:
        return [(r, a, c, b) for (c, b) in cs for (r, a) in rs]
    return [(r, a, c, b) for (r, a) in rs for (c, b) in cs]


@jax.jit
def pallas_sequential_preLN__sliding_block_cached__mixer_s_mlp__decode_kernel(
    A_x: jax.Array,
    A_k_cache: jax.Array,
    A_v_cache: jax.Array,
    A_wq: jax.Array,
    A_wo: jax.Array,
    B_x: jax.Array,
    B_w1: jax.Array,
    B_w2: jax.Array,
    B_w3: jax.Array,
    B_w4: jax.Array,
):
    B, S, D = A_x.shape
    _, Hkv, Sk, Dh = A_k_cache.shape
    H = _HQ
    F = B_w3.shape[1]
    W = min(4096, max(256, Sk // 4))
    assert B == 1 and S == 1, "decode kernel: one token"
    assert H % Hkv == 0 and A_wq.shape == (D, H * Dh) and A_wo.shape == (H * Dh, D)
    rep = H // Hkv
    nbuf = _NBUF
    w4_split = (768, 384, 256, 128) if F == 1536 else (F,)
    nw4 = len(w4_split)
    w4_off = [sum(w4_split[:i]) for i in range(nw4)]
    last_kv = H - nbuf - 1
    scale = Dh ** -0.5
    k_tiles = _tiles(Dh, W, 8, 2048, col_major=True, row_stride=3)
    v_tiles = _tiles(Dh, W, 32, 512, col_major=True)

    def kernel_function(x_hbm, kt_hbm, vt_hbm, wq_hbm, wo_hbm, w3_hbm, w4_hbm, o_ref,
                        x_v, kbuf, vbuf, wq_v, wo_v, w3_v, w4_v, q_scr,
                        ksem, vsem, wsem, w4sem):
        def piece(src, dst, sem, r, nr, c, nc):
            if nc == src.shape[1]:
                return pltpu.make_async_copy(src.at[pl.ds(r, nr)], dst.at[pl.ds(r, nr)], sem)
            return pltpu.make_async_copy(src.at[pl.ds(r, nr), pl.ds(c, nc)],
                                         dst.at[pl.ds(r, nr), pl.ds(c, nc)], sem)

        def start_two(list0, list1):
            i0 = i1 = 0
            while i0 < len(list0) or i1 < len(list1):
                if i1 >= len(list1) or (i0 < len(list0) and i0 * len(list1) <= i1 * len(list0)):
                    list0[i0].start(priority=0)
                    i0 += 1
                else:
                    list1[i1].start(priority=1)
                    i1 += 1

        def start_kv(h, slot):
            start_two(
                [pltpu.make_async_copy(
                    kt_hbm.at[0, h // rep, pl.ds(r, nr), pl.ds(Sk - W + c, nc)],
                    kbuf.at[slot, pl.ds(r, nr), pl.ds(c, nc)], ksem.at[slot])
                 for (r, nr, c, nc) in k_tiles],
                [pltpu.make_async_copy(
                    vt_hbm.at[0, h // rep, pl.ds(r, nr), pl.ds(Sk - W + c, nc)],
                    vbuf.at[slot, pl.ds(r, nr), pl.ds(c, nc)], vsem.at[slot])
                 for (r, nr, c, nc) in v_tiles])

        def split(lst, frac):
            n = int(round(len(lst) * frac))
            return lst[:n], lst[n:]

        def wait_all(buf, sem):
            pltpu.make_async_copy(buf, buf, sem).wait()

        x_cp = pltpu.make_async_copy(x_hbm.at[0], x_v, wsem.at[0])
        wq_p = [piece(wq_hbm, wq_v, wsem.at[1], *t)
                for t in _tiles(D, H * Dh, 8, 2048, True, row_stride=16)]
        wo_p = [piece(wo_hbm, wo_v, wsem.at[2], *t)
                for t in _tiles(H * Dh, D, 16, D, row_stride=96)]
        w3_p = [piece(w3_hbm, w3_v, wsem.at[3], *t)
                for t in _tiles(D, F, 32, 512, True, row_stride=4)]
        w4_p = [[piece(w4_hbm, w4_v, w4sem.at[c], *t)
                 for t in _tiles(w4_split[c], D, 16, D, r0=w4_off[c])] for c in range(nw4)]

        x_cp.start()
        start_two(wq_p, wo_p)

        def prime(s, carry):
            start_kv(s, s)
            return carry
        lax.fori_loop(0, nbuf, prime, 0)

        x_cp.wait()
        x = x_v[...].astype(jnp.float32)
        xn = _layernorm(x).astype(jnp.bfloat16)
        wait_all(wq_v, wsem.at[1])
        q = jnp.dot(xn, wq_v[...], preferred_element_type=jnp.float32).astype(jnp.bfloat16)
        for h in range(H):
            q_scr[h] = q[:, h * Dh:(h + 1) * Dh]

        def body(h, acc):
            slot = lax.rem(h, nbuf)
            wait_all(kbuf.at[slot], ksem.at[slot])
            s = jnp.dot(q_scr[h], kbuf[slot], preferred_element_type=jnp.float32) * scale
            m = jnp.max(s, axis=-1, keepdims=True)
            p = jnp.exp(s - m)
            l = jnp.sum(p, axis=-1, keepdims=True)
            wait_all(vbuf.at[slot], vsem.at[slot])
            o = lax.dot_general(p.astype(jnp.bfloat16), vbuf[slot], (((1,), (1,)), ((), ())),
                                preferred_element_type=jnp.float32)

            @pl.when(h + nbuf < H)
            def _():
                start_kv(h + nbuf, slot)

            @pl.when(h == min(last_kv + 1, H - 1))
            def _():
                start_two(*split(w3_p, _W3_FRAC))

            @pl.when(h == min(last_kv + 2, H - 1))
            def _():
                for c in range(nw4):
                    start_two(*split(w4_p[c], _W4_FRAC))

            @pl.when(h == 0)
            def _():
                wait_all(wo_v, wsem.at[2])

            o = (o / l).astype(jnp.bfloat16)
            r0 = pl.multiple_of(h * Dh, 16)
            return acc + jnp.dot(o, wo_v[pl.ds(r0, Dh), :], preferred_element_type=jnp.float32)

        a = lax.fori_loop(0, H, body, jnp.zeros((1, D), jnp.float32))

        h1 = x + a
        xb = _layernorm(h1)
        x1 = xb
        x1n = _layernorm(x1).astype(jnp.bfloat16)
        wait_all(w3_v, wsem.at[3])
        g = _gelu(jnp.dot(x1n, w3_v[...], preferred_element_type=jnp.float32)).astype(jnp.bfloat16)
        res = h1 + x1
        vpu_tail = nw4 > 1 and w4_split[-1] == 128 and D % 128 == 0
        if vpu_tail:
            g_col = jnp.broadcast_to(g[:, F - 128:].astype(jnp.float32), (128, 128)).T
        for c in range(nw4):
            rows = pl.ds(w4_off[c], w4_split[c])
            wait_all(w4_v.at[rows], w4sem.at[c])
            if vpu_tail and c == nw4 - 1:
                w = w4_v[rows, :].astype(jnp.float32)
                res = res + jnp.concatenate(
                    [jnp.sum(w[:, j:j + 128] * g_col, axis=0, keepdims=True)
                     for j in range(0, D, 128)], axis=1)
            else:
                res = res + jnp.dot(g[:, w4_off[c]:w4_off[c] + w4_split[c]], w4_v[rows, :],
                                    preferred_element_type=jnp.float32)
        o_ref[0] = res.astype(o_ref.dtype)

    kt = jnp.swapaxes(A_k_cache, 2, 3)
    vt = jnp.swapaxes(A_v_cache, 2, 3)
    any_spec = pl.BlockSpec(memory_space=pl.ANY)
    return pl.pallas_call(
        kernel_function,
        out_shape=jax.ShapeDtypeStruct((B, S, D), A_x.dtype),
        in_specs=[any_spec] * 7,
        out_specs=pl.BlockSpec(memory_space=pltpu.VMEM),
        scratch_shapes=[
            pltpu.VMEM((1, D), A_x.dtype),
            pltpu.VMEM((nbuf, Dh, W), A_k_cache.dtype),
            pltpu.VMEM((nbuf, Dh, W), A_v_cache.dtype),
            pltpu.VMEM((D, H * Dh), A_wq.dtype),
            pltpu.VMEM((H * Dh, D), A_wo.dtype),
            pltpu.VMEM((D, F), B_w3.dtype),
            pltpu.VMEM((F, D), B_w4.dtype),
            pltpu.VMEM((H, 1, Dh), jnp.bfloat16),
            pltpu.SemaphoreType.DMA((nbuf,)),
            pltpu.SemaphoreType.DMA((nbuf,)),
            pltpu.SemaphoreType.DMA((4,)),
            pltpu.SemaphoreType.DMA((nw4,)),
        ],
        compiler_params=pltpu.CompilerParams(vmem_limit_bytes=64 * 1024 * 1024),
    )(A_x, kt, vt, A_wq, A_wo, B_w3, B_w4)
```
